```python
import os as _os
_os.environ.setdefault("JAX_PLATFORMS", "cpu")
import jax
import jax.numpy as jnp

def _softmax(x, axis=-1):
    return jax.nn.softmax(x, axis=axis)
def _gelu(x):
    return jax.nn.gelu(x, approximate=True)
def _silu(x):
    return jax.nn.silu(x)
def _sigmoid(x):
    return jax.nn.sigmoid(x)
def _layernorm(x, axis=-1, eps=1e-5):
    m = jnp.mean(x, axis=axis, keepdims=True)
    v = jnp.var(x, axis=axis, keepdims=True)
    return (x - m) / jnp.sqrt(v + eps)
def _scatter_add(tgt, idx, src, axis=0):
    return tgt.at[idx].add(src)
def _segment_sum(src, seg, n):
    return jax.ops.segment_sum(src, seg, n)
class _Rng:
    def __init__(self, key):
        self._k = key
    def _next(self):
        self._k, sub = jax.random.split(self._k)
        return sub
    def normal(self, shape):
        return jax.random.normal(self._next(), shape, dtype=jnp.bfloat16)
    def randint(self, lo, hi, shape):
        return jax.random.randint(self._next(), shape, lo, hi, dtype=jnp.int32)
    def uniform(self, shape, lo=0.0, hi=1.0):
        return jax.random.uniform(self._next(), shape, jnp.bfloat16, lo, hi)
    def permutation(self, n):
        return jax.random.permutation(self._next(), n)


kernel_name = 'parallel_sum__sliding_local_dilated__geglu_ffn__prompt'

def setup_inputs():
    _rng = _Rng(jax.random.key(int.from_bytes(__import__("os").urandom(4), "little")))
    _w = (lambda a: (lambda t: t.astype(jnp.bfloat16) if jnp.issubdtype(t.dtype, jnp.floating) else t)(jnp.asarray(a)))
    def _A_setup():
        B, S, D = 1, 2048, 640
        return {
            "x": _w((lambda *s: _rng.normal(s) * 0.05)(B, S, D)),
            "wqkv": _w((lambda *s: _rng.normal(s) * 0.05)(D, 3 * D)),
            "wo": _w((lambda *s: _rng.normal(s) * 0.05)(D, D)),
        }
    _A_in = _A_setup()

    def _B_setup():
        B, S, D, F = 1, 2048, 640, 1728
        return {
            "x": _w((lambda *s: _rng.normal(s) * 0.05)(B, S, D)),
            "w_gate": _w((lambda *s: _rng.normal(s) * 0.05)(D, F)),
            "w_up": _w((lambda *s: _rng.normal(s) * 0.05)(D, F)),
            "w_down": _w((lambda *s: _rng.normal(s) * 0.05)(F, D)),
        }
    _B_in = _B_setup()

    return {
        "A_x": _A_in["x"],
        "A_wqkv": _A_in["wqkv"],
        "A_wo": _A_in["wo"],
        "B_x": _B_in["x"],
        "B_w_gate": _B_in["w_gate"],
        "B_w_up": _B_in["w_up"],
        "B_w_down": _B_in["w_down"],
    }

def reference(A_x, A_wqkv, A_wo, B_x, B_w_gate, B_w_up, B_w_down):
    def _A_ref(x, wqkv, wo):
        B, S, D = x.shape
        H = 32; Dh = D // H
        W, dil = 8, 2
        qkv = (lambda x, *d: x.transpose(*d))((x @ wqkv).reshape(B, S, 3, H, Dh), 2, 0, 3, 1, 4)
        q, k, v = qkv[0], qkv[1], qkv[2]
        scale = Dh ** -0.5
        pos = jnp.arange(S)
        off = jnp.arange(W) * dil
        idx = pos[:, None] - off[None, :]
        mask = idx >= 0
        idx_c = jnp.where(mask, idx, 0).reshape(-1)
        kg = k[:, :, idx_c, :].reshape(B, H, S, W, Dh)
        vg = v[:, :, idx_c, :].reshape(B, H, S, W, Dh)
        logits = jnp.einsum("bhsd,bhswd->bhsw", q, kg) * scale
        logits = jnp.where(mask[None, None, :, :], logits, -1e9)
        attn = _softmax(logits, axis=-1)
        o = jnp.einsum("bhsw,bhswd->bhsd", attn, vg)
        return (lambda x, *d: x.transpose(*d))(o, 0, 2, 1, 3).reshape(B, S, D) @ wo

    def _B_ref(x, w_gate, w_up, w_down):
        return (_gelu(x @ w_gate) * (x @ w_up)) @ w_down

    x = A_x
    xn = _layernorm(x, axis=-1)
    return x + _A_ref(xn, A_wqkv, A_wo) + _B_ref(xn, B_w_gate, B_w_up, B_w_down)
```

```python
import functools
import numpy as np
import jax
import jax.numpy as jnp
from jax import lax
import jax.experimental.pallas as pl
import jax.experimental.pallas.tpu as pltpu

S, D, F = 2048, 640, 1728
H, DH, W, DIL = 32, 20, 8, 2
L = 128
NT = D // L
HALO = 16
f32, bf16, u32 = jnp.float32, jnp.bfloat16, jnp.uint32
LOG2E = 1.4426950408889634

TM = 256
NB, P = S // TM, TM // 2
RC, RS, RA = 16, 8, 8
NS = 3
TS = 4
N0 = 3
XS = (0, 1, 2, 4, 8)
RATES = (62, 60, 74, 76)
LAG0, LAG, DELAY = 2, 5, 4
PERIOD = (4, 2)
EARLY = dict(K=6, V=6, Q=9, U0=9, U1=9, GU=13, GL=13, O=13, D0=13, D1=13, D2=13)
STAGES = ("U0", "K", "V", "Q", "U1", "GU", "GL", ("D0", "D1"), ("D2",), ("O",))


def _scheme(nn):
    nk = 5
    pts = np.array([[1, 0], [0, 1], [-1, -1]])
    ann = np.array([[-p[1], p[0]] for p in pts])
    ek, en = np.eye(nk, dtype=int), np.eye(nn, dtype=int)
    prods = {}

    def term(a, o, w):
        sa = np.sign(a.ravel()[np.flatnonzero(a)[0]])
        so = np.sign(o.ravel()[np.flatnonzero(o)[0]])
        key = (tuple((a * sa).ravel()), tuple((o * so).ravel()))
        prods[key] = prods.get(key, 0) + w * sa * so

    def diag(k, n, ty, w):
        p, q = [i for i in range(3) if i != ty]
        for i, j in ((p, q), (q, p)):
            term(np.outer(pts[i], k), np.outer(ann[j], n) * int(ann[j] @ pts[i]), w)

    def pair(ki, ni, ti, kj, nj, tj, wij, wji):
        z = 3 - ti - tj
        ui, uj = pts[tj], -pts[ti]
        fi, fj = ann[tj] * int(ann[tj] @ pts[z]), ann[ti] * int(ann[ti] @ pts[z])
        eta = ann[z] * int(ann[z] @ ui)
        term(np.outer(uj, ki - kj), np.outer(fi, nj - ni), wij)
        term(np.outer(ui, kj - ki), np.outer(fj, ni - nj), -wji)
        term(np.outer(ui, ki) - np.outer(uj, kj), np.outer(fi, ni) - np.outer(fj, nj), wij - wji)
        term(np.outer(pts[z], ki), np.outer(fi, ni), wij)
        term(np.outer(uj, kj), np.outer(eta, nj), wij)
        term(np.outer(pts[z], kj), np.outer(fj, nj), wji)
        term(np.outer(ui, ki), np.outer(eta, ni), wji)

    w = {(k, n): np.outer(ek[k], en[n]) for k in range(nk) for n in range(nn)}
    ty = (0, 0, 1, 1, 2)
    if nn == 2:
        for a, b in ((0, 2), (1, 3)):
            diag(ek[a], en[0], ty[a], w[a, 0])
            diag(ek[b], en[1], ty[b], w[b, 1])
            pair(ek[a], en[0], ty[a], ek[b], en[1], ty[b], w[a, 1], w[b, 0])
        for n in range(2):
            diag(ek[4], en[n], ty[4], w[4, n])
    else:
        for i in range(5):
            diag(ek[i], en[i], ty[i], w[i, i])
        for i, j, h in ((0, 1, 2), (3, 2, 1)):
            pair(ek[i], en[i], ty[i], ek[j] - ek[h], en[j] - en[h], 3 - ty[j] - ty[h], w[i, j], w[j, i])
            w[i, h], w[h, i] = w[i, h] + w[i, j], w[h, i] + w[j, i]
        for i in range(5):
            for j in range(i + 1, 5):
                if ty[i] != ty[j]:
                    pair(ek[i], en[i], ty[i], ek[j], en[j], ty[j], w[i, j], w[j, i])
    U = np.array([k[0] for k in prods]).reshape(-1, 2, nk)
    O = np.array([k[1] for k in prods]).reshape(-1, 2, nn)
    V = np.array(list(prods.values()))
    ref = np.einsum("ab,cd,ef->acdebf", np.eye(2), np.eye(nk), np.eye(nn))
    assert np.array_equal(np.einsum("rac,rde,rbf->acdebf", U, V, O), ref)
    assert max(np.abs(t).max() for t in (U, V, O)) == 1
    return U, V, O


def _plan(rows):
    sums = [{int(i): int(r[i]) for i in np.flatnonzero(r)} for r in rows]
    steps, nxt = [], rows.shape[1]
    while True:
        count = {}
        for s in sums:
            ks = sorted(s)
            for x, a in enumerate(ks):
                for b in ks[x + 1:]:
                    key = (a, b, s[a] * s[b])
                    count[key] = count.get(key, 0) + 1
        best = max(count.items(), key=lambda kv: (kv[1], -kv[0][1], -kv[0][0]), default=(None, 0))
        if best[1] < 2:
            return steps, [sorted(s.items()) for s in sums]
        a, b, sg = best[0]
        steps.append((a, b, sg))
        for s in sums:
            if a in s and b in s and s[a] * s[b] == sg:
                s[nxt] = s[a]
                del s[a], s[b]
        nxt += 1

def _signed_sums(plan, get, reload=False):
    steps, sums, n_in = plan
    memo, ops = {}, [0]

    def val(i):
        if reload and i < n_in:
            return get(i)
        if i not in memo:
            if i < n_in:
                memo[i] = get(i)
            else:
                a, b, sg = steps[i - n_in]
                memo[i] = val(a) + val(b) if sg > 0 else val(a) - val(b)
                ops[0] += 1
        return memo[i]

    for s in sums:
        s = sorted(s, key=lambda t: t[1] < 0)
        acc = val(s[0][0]) if s[0][1] > 0 else -val(s[0][0])
        for i, sg in s[1:]:
            acc = acc + val(i) if sg > 0 else acc - val(i)
        yield acc, (ops[0] + len(s) - 1) * (acc.shape[0] // 8)
        ops[0] = 0


class _Algo:
    def __init__(self, nn=5, drop=None, acts=None):
        U, V, O = _scheme(nn)
        for r in range(len(V)):
            if (V[r] <= 0).all():
                V[r], O[r] = -V[r], -O[r]
        if drop is not None:
            U[:, :, drop], V[:, drop, :] = 0, 0
        self.nn, self.n = nn, len(U)
        self.live = [r for r in range(self.n) if U[r].any() and V[r].any()]
        self.acts = {} if acts is None else acts
        self.act = {r: self.acts.setdefault(tuple(U[r].ravel()), len(self.acts)) for r in self.live}
        self.plain = {r: tuple(int(i) for i in np.argwhere(V[r])[0]) for r in self.live
                      if np.abs(V[r]).sum() == 1 and V[r].sum() > 0}
        self.mixed = {r: i for i, r in enumerate(r for r in self.live if r not in self.plain)}
        slots = {}
        for r in range(self.n):
            slots.setdefault(tuple(O[r].ravel()), []).append(r)
        self.slots = [[r for r in rs if r in self.live] for rs in slots.values()]
        self.w_plan = _plan(V[list(self.mixed)].reshape(len(self.mixed), 5 * nn)) + (5 * nn,)
        self.out_plan = _plan(np.array(list(slots)).T) + (len(slots),)

    def act_plan(self):
        return _plan(np.array(list(self.acts))) + (10,)


def _geglu2(g, u):
    c = 0.7978845608028654
    return (1.0 + jnp.tanh(g * (c + (c * 0.044715) * (g * g)))) * (g * u)


def _pack(x):
    return pltpu.pack_elementwise([x[:len(x) // 2], x[len(x) // 2:]], packed_dtype=bf16)


def _unpack(words):
    return jnp.concatenate([pltpu.bitcast(words << 16, f32), pltpu.bitcast(words & np.uint32(0xFFFF0000), f32)])


class _Pacer:
    def __init__(self, zero, rate, lag, every):
        self.every = every
        self.zero, self.rate, self.lag = zero.astype(u32), rate, lag
        self.jobs, self.running, self.due, self.budget, self.n = [], None, [], 0, 0

    def add(self, group, deadline, gens, after=(), delay=0):
        self.jobs += [(deadline, group, after, self.n + delay, g) for g in gens]

    def _pick(self, urgent):
        busy = [j[1] for j in self.jobs]
        ok = [j for j in self.jobs if not any(a in busy for a in j[2]) and (urgent or j[3] <= self.n)]
        return min(ok, key=lambda j: j[0], default=None)

    def _advance(self, urgent=False):
        self.running = self.running or self._pick(urgent)
        if self.running is None:
            return None
        step = next(self.running[4], None)
        if step is None:
            self.jobs = [j for j in self.jobs if j is not self.running]
            self.running = None
            return None, 0
        return step

    def finish(self, deadline):
        while any(j[0] <= deadline for j in self.jobs):
            self._advance(True)

    def pace(self, words):
        self.n += 1
        rows = [words[r:r + 8] for r in range(0, len(words), 8)]
        for j in range(self.every):
            self.budget, newest = min(self.budget, 0) + self.rate // self.every, None
            while self.budget > 0:
                step = self._advance()
                if step is None:
                    break
                newest = newest if step[0] is None else step[0]
                self.budget -= step[1]
            self.due.append(newest)
            v = self.due.pop(0) if len(self.due) > self.lag * self.every else None
            if v is not None:
                v = v if v.dtype == u32 else pltpu.bitcast(v, u32)
                at = ((self.n - 1) % 4 * self.every + j) * len(rows) // (4 * self.every)
                rows[at] |= (v if len(v) == 8 else v[:8] | v[8:]) & self.zero
        return jnp.concatenate(rows)


def _once(fn, *args):
    fn(*args)
    yield None, 0


LAYER2 = ("D0", "D1", "D2", "O")
FEEDS = {"G0": "U0", "G1": "U1", "GU": "GL", "U0": "D0", "U1": "D1", "GL": "D2", "Q": "O", "K": "O", "V": "O"}


def _kernel(x_hbm, wqkv_hbm, wo_hbm, wg_hbm, wu_hbm, wd_hbm, out_hbm,
            x_v, out_v, wqkv_raw, wqkv_v, wo_raw, wo_v, wg_v, wgu_v, wd_v, a1_v, p1_v, p2_v, stat_v, xn_v,
            wmix, res, in_sems, out_sems, zero_s, *, algo):
    chunks = range(0, P, RC)
    zero_s[0] = 0

    def slabs(hbm, r0, n, vmem, v0, c0=0):
        if len(vmem.shape) == 2:
            cols = pl.ds(c0 * L, D)
            return [(hbm.bitcast(u32).at[pl.ds(r0 // 2, n // 2), cols], vmem.at[pl.ds(v0 // 2, n // 2), cols])]
        return [(hbm.bitcast(u32).at[pl.ds(r0 // 2, n // 2), pl.ds((c0 + t) * L, L)],
                 vmem.at[c0 + t, pl.ds(v0 // 2, n // 2), :]) for t in range(NT)]
    gate = lambda r0, n: [(wg_hbm.at[pl.ds(r0, n), :], wg_v.at[pl.ds(r0, n), :])]
    loads = {
        "G0": gate(0, N0 * L), "G0b": gate(N0 * L, D - N0 * L),
        "U0": slabs(wu_hbm, 0, D, wgu_v, 0),
        "G1": gate(D, D), "U1": slabs(wu_hbm, D, D, wgu_v, D),
        "GU": slabs(wg_hbm, 2 * D, 3 * L, wgu_v, 10 * L) + slabs(wu_hbm, 2 * D, 2 * L, wgu_v, 13 * L),
        "GL": (slabs(wu_hbm, 12 * L, L, wgu_v, 15 * L) + slabs(wg_hbm, 13 * L, 64, wgu_v, 16 * L)
               + slabs(wu_hbm, 13 * L, 64, wgu_v, 16 * L + 64)),
        "Q": slabs(wqkv_hbm, 0, D, wqkv_raw, 0), "K": slabs(wqkv_hbm, 0, D, wqkv_raw, 0, NT),
        "V": slabs(wqkv_hbm, 0, D, wqkv_raw, 0, 2 * NT),
        "D0": slabs(wd_hbm, 0, D, wd_v, 0), "D1": slabs(wd_hbm, D, D, wd_v, D),
        "D2": slabs(wd_hbm, 2 * D, F - 2 * D, wd_v, 2 * D), "O": slabs(wo_hbm, 0, D, wo_raw, 0),
    }
    loads.update({b: [c for j in range(b, e) for c in slabs(x_hbm, j * TM, TM, x_v.at[j], 0)]
                  for b, e in zip(XS, XS[1:])})
    copies = {name: [pltpu.make_async_copy(s, d, in_sems.at[i]) for s, d in pairs]
              for i, (name, pairs) in enumerate(loads.items())}

    def start(*names):
        for name in names:
            for c in copies[name]:
                c.start()

    def wait(name):
        for c in copies[name]:
            c.wait()

    def gu_tile(t0):
        return lambda k, n: wgu_v.at[pl.ds((t0 + n) * 64, 64), pl.ds(k * L, L)]
    raw = {
        "U0": gu_tile(0), "U1": gu_tile(5), "GU": gu_tile(10), "GL": gu_tile(15),
        "Q": lambda k, n: wqkv_v.at[n, pl.ds(k * 64, 64), :],
        "K": lambda k, n: wqkv_v.at[5 + n, pl.ds(k * 64, 64), :],
        "V": lambda k, n: wqkv_v.at[10 + n, pl.ds(k * 64, 64), :],
        "D0": lambda k, n: wd_v.at[pl.ds(k * 64, 64), pl.ds(n * L, L)],
        "D1": lambda k, n: wd_v.at[pl.ds((5 + k) * 64, 64), pl.ds(n * L, L)],
        "D2": lambda k, n: wd_v.at[pl.ds((9 + k) * 64, 64), pl.ds(n * L, L)],
        "O": lambda k, n: wo_v.at[n, pl.ds(k * 64, 64), :],
    }

    def mix_rows(name, c):
        half = pl.ds(c * 8, 8)
        get = lambda i: _unpack(raw[name](*divmod(i, algo[name].nn))[half, :])
        for i, (val, ops) in enumerate(_signed_sums(algo[name].w_plan, get)):
            wmix[name][i, half, :] = words = _pack(val)
            yield words, ops + 1

    def permute_qkv(p, k, c):
        lane = lax.broadcasted_iota(jnp.int32, (8, L), 1)
        src = [wqkv_raw[pl.ds(k * 64 + c * 8, 8), pl.ds(p * D + j * L, L)] for j in range(NT)]
        lm5 = lane - 5 * ((lane * 52) >> 8)
        lm5 = jnp.where(lm5 < 0, lm5 + 5, lm5)
        base = (lane & 31) * 20 + (lane >> 5) * 5
        for t in range(NT):
            m = src[0]
            for j in range(1, NT):
                m = jnp.where(lm5 == (t - 3 * j) % 5, src[j], m)
            m = jnp.take_along_axis(m, (base + t) & (L - 1), axis=1, mode="promise_in_bounds")
            wqkv_v[p * NT + t, pl.ds(k * 64 + c * 8, 8), :] = m
        yield None, 30

    def permute_wo(c):
        for j in range(NT):
            for t in range(NT):
                src = 5 * (c // 2) + 320 * (c % 2) + t
                a, b = [wo_raw[j, pl.ds(src // 2 + o, 8, stride=20), :] for o in (0, 10)]
                wo_v[j, pl.ds(t * 64 + c * 8, 8), :] = ((a >> 16) | (b & np.uint32(0xFFFF0000)) if src % 2 else
                                                        (a & np.uint32(0xFFFF)) | (b << 16))
            yield None, 20

    def prep(names):
        jobs = [permute_qkv("QKV".index(n), k, c) for n in names if n in ("Q", "K", "V") for c in range(8) for k in range(NT)]
        jobs += [permute_wo(c) for c in range(8) if "O" in names]
        return jobs + [mix_rows(n, c) for n in names for c in range(8)]

    def product(pacer, name, acts, r):
        w = raw[name](*algo[name].plain[r])[...] if r in algo[name].plain else wmix[name][algo[name].mixed[r]]
        w = pltpu.bitcast(w, bf16)
        return lax.dot_general(pltpu.bitcast(pacer.pace(acts[algo[name].act[r]]), bf16), w,
                               (((1,), (1 if name[0] in "GU" else 0,)), ((), ())), preferred_element_type=f32)

    def result(name, b):
        return res[name].at[b if res[name].shape[0] > 1 else 0]

    def store_acts(ref, plan, tiles, r0):
        for i, (val, ops) in enumerate(_signed_sums(plan, lambda j: tiles[j])):
            ref[i, pl.ds(r0 // 2, RC // 2), :] = words = _pack(val)
            yield words, ops + 1

    act_plans = {n: algo[n].act_plan() for n in ("Q",) + LAYER2}

    def x_rows(b, r):
        return [_unpack(x_v[b, pl.ds(r // 2, RC // 2), pl.ds(t * L, L)]) for t in range(NT)]

    def normed(b, r):
        mean, inv = stat_v[b, 0, pl.ds(r, RC), :], stat_v[b, 1, pl.ds(r, RC), :]
        return [(x - mean) * inv for x in x_rows(b, r)]

    def norm(b):
        def row_mean(tiles):
            part = functools.reduce(jnp.add, tiles)
            return part, jnp.broadcast_to(jnp.sum(part, axis=-1, keepdims=True) * (1.0 / D), (RC, L))

        def center(r):
            part, stat_v[b, 0, pl.ds(r, RC), :] = row_mean(x_rows(b, r))
            yield part, 22

        def spread(r):
            mean = stat_v[b, 0, pl.ds(r, RC), :]
            part, var = row_mean([jnp.square(x - mean) for x in x_rows(b, r)])
            stat_v[b, 1, pl.ds(r, RC), :] = lax.rsqrt(var + 1e-5)
            yield part, 56

        def apply(r):
            for t, val in enumerate(normed(b, r)):
                xn_v[t, pl.ds(b * P + r // 2, RC // 2), :] = _pack(val)
            yield val, 35
        return [job(r) for job in (center, spread, apply) for r in range(0, TM, RC)]

    def input_sums(b, r0):
        tiles = []
        for m in range(2):
            tiles += normed(b, m * P + r0)
            yield tiles[-1], 35
        yield from store_acts(a1_v.at[b], act_plans["Q"], tiles, r0)

    def outputs(name, slot, r0, n):
        return enumerate(_signed_sums(algo[name].out_plan, lambda r: p1_v[slot, r, pl.ds(r0, n), :], reload=True))

    def to_tiles(name, slot, b, r0):
        for r in range(r0, r0 + RC, RS):
            for i, (val, ops) in outputs(name, slot, r, RS):
                if name in ("K", "V"):
                    res[name][i % NT, pl.ds(HALO + (i // NT) * P + r, RS), :] = val
                else:
                    result(name, b)[i, pl.ds(r, RS), :] = val * (DH ** -0.5 * LOG2E) if name == "Q" else val
                yield val, ops

    def to_hidden(name, slot, b, r0):
        parts = []
        for r in range(r0, r0 + RC, RS):
            gate = lambda i: result({"U0": "G0", "U1": "G1", "GL": "GU"}[name], b)[i, pl.ds(r, RS), :]
            tiles = []
            for i, (up, ops) in outputs(name, slot, r, RS):
                if name != "GL":
                    tiles.append(_geglu2(gate(i), up))
                elif i % 2 == 0:
                    m = 5 * (i // 2)
                    tiles.append(None)
                    for j in range(2):
                        tiles.append(_geglu2(gate(m + j), gate(m + 3 + j)))
                        yield tiles[-1], RS
                    tiles.append(_geglu2(gate(m + 2), up))
                else:
                    low = lax.broadcasted_iota(jnp.int32, (RS, L), 1) < 64
                    tiles.append(jnp.where(low, _geglu2(up, pltpu.roll(up, 64, 1)), 0.0))
                yield tiles[-1], ops + RS
            parts.append(tiles)
        tiles = [None if p[0] is None else jnp.concatenate(p) for p in zip(*parts)]
        yield from store_acts(result(name, b), act_plans[FEEDS[name]], tiles, r0)

    def post(name, slot, b):
        return [(to_hidden if name in ("U0", "U1", "GL") else to_tiles)(name, slot, b, r0) for r0 in chunks]

    def halo(b, keep):
        for ref in (res["K"], res["V"]):
            for t in range(NT):
                ref[t, :HALO] = (ref[t, TM:TM + HALO] if keep else
                                 jnp.where(b > 0, ref[t, :HALO], jnp.broadcast_to(ref[t, HALO:HALO + 1], (HALO, L))))

    def attend(b):
        steps = [j + k for j in range(W // 2) for k in (0, W // 2)]
        held = {}

        def windows(name, row):
            span = functools.cache(lambda t, j: res[name][t, pl.ds(HALO + row - 8 - DIL * j, RA + 8), :])
            return lambda t, w: span(t, w % 4)[8 - w // 4 * 8:][:RA]

        def score(m, r):
            row, k = m * P + r, windows("K", m * P + r)
            q = [result("Q", b)[m * NT + t, pl.ds(r, RA), :] for t in range(NT)]
            for w in steps:
                part = functools.reduce(jnp.add, [q[t] * k(t, w) for t in range(NT)])
                s = part + pltpu.roll(part, 64, 1)
                s = s + pltpu.roll(s, 32, 1)
                if row < DIL * w:
                    s = jnp.where(b * TM + row + lax.broadcasted_iota(jnp.int32, (RA, L), 0) >= DIL * w, s, -1e9 * LOG2E)
                held[row, w] = s
                yield part, 11 * RA // 8

        def mix(m, r, tiles):
            row, v = m * P + r, windows("V", m * P + r)
            logits = [held[row, w] for w in steps]
            top = functools.reduce(jnp.maximum, logits)
            e = [jnp.exp2(s - top) for s in logits]
            inv = 2.0 / functools.reduce(jnp.add, e)
            yield top, 30 * RA // 8
            for t in range(NT):
                part = functools.reduce(jnp.add, [p * v(t, w) for p, w in zip(e, steps)])
                tiles[m * NT + t].append(inv * part)
                yield part, 16 * RA // 8

        def chunk(r0):
            pieces = [(m, r) for m in range(2) for r in range(r0, r0 + RC, RA)]
            tiles = [[] for _ in range(2 * NT)]
            yield from score(*pieces[0])
            for i, piece in enumerate(pieces):
                if i + 1 < len(pieces):
                    yield from score(*pieces[i + 1])
                yield from mix(*piece, tiles)
            yield from store_acts(result("att", b), act_plans["O"], [jnp.concatenate(t) for t in tiles], r0)
        return [chunk(r0) for r0 in chunks]

    def finish(b, r0):
        weave = lambda v: pltpu.bitcast(_pack(v), bf16).astype(f32)
        sums = _signed_sums(algo["O"].out_plan, lambda r: p2_v[r, pl.ds(r0, RC), :], reload=True)
        for i, (val, ops) in enumerate(sums):
            at = b, pl.ds(((i // NT) * P + r0) // 2, RC // 2), pl.ds(i % NT * L, L)
            y = weave(pltpu.bitcast(x_v[at], bf16).astype(f32)) + 0.5 * val
            out_v[b, pl.ds((i // NT) * P + r0, RC), at[2]] = _unpack(pltpu.bitcast(y.astype(bf16), u32)).astype(bf16)
            yield y, ops + 16

    def out_copy(b, r0, n, i):
        start = b * TM + r0 if isinstance(b, int) else pl.multiple_of(b * TM + r0, n)
        return pltpu.make_async_copy(
            out_v.at[b, pl.ds(r0, n), :], out_hbm.at[pl.ds(start, n), :], out_sems.at[i])

    def send(b, prev):
        pl.when(b > 0)(out_copy(prev, 0, TM, prev).start)
        out_v[b, :RC, :L] = jnp.zeros((RC, L), bf16)
        yield out_v[b + zero_s[0], :RC, :L], 10 ** 2

    def drain(jobs):
        for job in jobs:
            for _ in job:
                pass

    start(0, "G0")
    wd_v[F // 2:] = jnp.zeros((32, D), u32)
    p2_v[...] = jnp.zeros(p2_v.shape, f32)
    for n in "KV":
        res[n][:, :HALO] = jnp.zeros((NT, HALO, L), f32)
    wait(0)
    start("G0b", XS[1])
    drain(norm(0))
    wait("G0")
    start(XS[2], "G1")
    todo = sorted((b + i, i, b) for i in range(2) for b in range(NB))
    when = {(i, b): t for t, (_, i, b) in enumerate(todo)}
    pacer = _Pacer(zero_s[0], RATES[0] * TM // L, LAG0, PERIOD[0])
    for t, (_, i, b) in enumerate(todo):
        ready = [n for n in EARLY if EARLY[n] == t]
        for n in ready + [XS[2], "G1"] * (t == when[1, 0]) + [XS[3]] * (t == when[1, XS[3] - 2]):
            wait(n)
        pacer.add("w", len(todo), prep(ready))
        if i == 1 and b + 2 < NB:
            pacer.add("norm", when[0, b + 2], norm(b + 2))
        if i == 1:
            pacer.add("sums", len(todo), [input_sums(b, r0) for r0 in chunks])
        pacer.finish(t)
        for n in range(NT):
            if t == 0 and n == N0:
                wait("G0b")
                wait(XS[1])
                start(XS[3], *EARLY)
                pacer.add("norm", 1, norm(1))
            g = functools.reduce(jnp.add, [lax.dot_general(
                pltpu.bitcast(pacer.pace(xn_v[k, pl.ds(b * TM // 2, TM // 2), :]), bf16),
                wg_v[pl.ds(i * D + n * L, L), pl.ds(k * L, L)],
                (((1,), (1,)), ((), ())), preferred_element_type=f32) for k in range(NT)])
            res["G%d" % i][b, n], res["G%d" % i][b, NT + n] = g[:P], g[P:]
    pacer.finish(len(todo))

    stages = STAGES
    at = {n: i for i, st in enumerate(stages) for n in (st if isinstance(st, tuple) else (st,))}
    n1, end = min(at[n] for n in LAYER2), len(stages)

    def block(b, carry):
        pacer = _Pacer(zero_s[0], 0, LAG, PERIOD[1])
        prev = jnp.maximum(b - 1, 0)
        pacer.add("out", n1, [finish(prev, r0) for r0 in chunks] + [send(b, prev)])
        for i, st in enumerate(stages):
            pacer.rate = RATES[1 + (i > max(at[n] for n in "QKV")) + (i >= n1)] * P // L
            if i == max(at[n] for n in "QKV") + 1:
                pacer.add("att", at["O"], [_once(halo, b, False)] + attend(b) + [_once(halo, b, True)], after=tuple("QKV"))
            pacer.finish(i)
            if i >= n1:
                for c in range(len(algo["O"].slots)):
                    vals = [product(pacer, n, result({"D0": "U0", "D1": "U1", "D2": "GL", "O": "att"}[n], b), r)
                            for n in st for r in algo[n].slots[c]]
                    if vals:
                        p2_v[c] = functools.reduce(jnp.add, vals + ([] if i == n1 else [p2_v[c]]))
                continue
            for c, rs in enumerate(algo[st].slots):
                p1_v[i % NS, c] = functools.reduce(jnp.add, [product(pacer, st, a1_v.at[b], r) for r in rs])
            pacer.add(st, min(i + NS, at[FEEDS[st]] if FEEDS[st] in LAYER2 else end), post(st, i % NS, b),
                      after=tuple(n for n in FEEDS if FEEDS[n] == st), delay=DELAY)
        pacer.finish(end)
    lax.fori_loop(0, NB, block, None)

    pending = [out_copy(b, 0, TM, b) for b in range(NB - 1)]
    for r0 in range(0, P, P // TS):
        drain(finish(NB - 1, r) for r in range(r0, r0 + P // TS, RC))
        for m in range(2):
            pending.append(out_copy(NB - 1, m * P + r0, P // TS, len(pending)))
            pending[-1].start()
    for c in pending:
        c.wait()


@jax.jit
def pallas_parallel_sum__sliding_local_dilated__geglu_ffn__prompt_kernel(
    A_x: jax.Array,
    A_wqkv: jax.Array,
    A_wo: jax.Array,
    B_x: jax.Array,
    B_w_gate: jax.Array,
    B_w_up: jax.Array,
    B_w_down: jax.Array,
):
    del B_x
    wide, deep = _Algo(), _Algo()
    algo = {n: wide for n in ("U0", "U1", "GU", "Q", "K", "V")}
    algo.update(GL=_Algo(nn=2, acts=wide.acts), D0=deep, D1=deep, D2=_Algo(drop=0), O=deep)
    sums = pltpu.VMEM((1, len(deep.acts), P // 2, L), u32)
    res = {"att": sums, "U0": sums, "U1": sums, "GL": sums}
    res.update({n: pltpu.VMEM((NT, 2 * HALO + TM, L), f32) for n in "KV"})
    res.update({n: pltpu.VMEM((blocks, 2 * NT, P, L), f32) for n, blocks in dict(G0=NB, G1=NB, GU=1, Q=1).items()})
    hbm = pl.BlockSpec(memory_space=pltpu.HBM)
    out = pl.pallas_call(
        functools.partial(_kernel, algo=algo),
        in_specs=[hbm] * 6,
        out_specs=hbm,
        out_shape=jax.ShapeDtypeStruct((S, D), bf16),
        scratch_shapes=[
            pltpu.VMEM((NB, P, D), u32), pltpu.VMEM((NB, TM, D), bf16),
            pltpu.VMEM((D // 2, 3 * D), u32), pltpu.VMEM((3 * NT, D // 2, L), u32),
            pltpu.VMEM((NT, D // 2 + 32, L), u32), pltpu.VMEM((NT, D // 2, L), u32),
            pltpu.VMEM((2 * D, D), bf16), pltpu.VMEM((17 * 64, D), u32), pltpu.VMEM((14 * 64, D), u32),
            pltpu.VMEM((NB, len(wide.acts), P // 2, L), u32),
            pltpu.VMEM((NS, len(wide.slots), P, L), f32), pltpu.VMEM((len(deep.slots), P, L), f32),
            pltpu.VMEM((NB, 2, TM, L), f32), pltpu.VMEM((NT, S // 2, L), u32),
            {n: pltpu.VMEM((len(a.mixed), L // 2, L), u32) for n, a in algo.items()}, res,
            pltpu.SemaphoreType.DMA((20,)), pltpu.SemaphoreType.DMA((NB + 2 * TS,)), pltpu.SMEM((1,), jnp.int32),
        ],
        compiler_params=pltpu.CompilerParams(vmem_limit_bytes=90 * 1024 * 1024),
    )(A_x.reshape(S, D), A_wqkv, A_wo, B_w_gate.T, B_w_up.T, B_w_down)
    return out.reshape(1, S, D)
```
